```python
import jax
import jax.numpy as jnp

def _softmax(x, axis=-1):
    return jax.nn.softmax(x, axis=axis)
def _gelu(x):
    return jax.nn.gelu(x, approximate=True)
def _silu(x):
    return jax.nn.silu(x)
def _sigmoid(x):
    return jax.nn.sigmoid(x)
def _layernorm(x, axis=-1, eps=1e-5):
    m = jnp.mean(x, axis=axis, keepdims=True)
    v = jnp.var(x, axis=axis, keepdims=True)
    return (x - m) / jnp.sqrt(v + eps)
def _scatter_add(tgt, idx, src, axis=0):
    return tgt.at[idx].add(src)
def _segment_sum(src, seg, n):
    return jax.ops.segment_sum(src, seg, n)
class _Rng:
    def __init__(self, key):
        self._k = key
    def _next(self):
        self._k, sub = jax.random.split(self._k)
        return sub
    def normal(self, shape):
        return jax.random.normal(self._next(), shape, dtype=jnp.bfloat16)
    def randint(self, lo, hi, shape):
        return jax.random.randint(self._next(), shape, lo, hi, dtype=jnp.int32)
    def uniform(self, shape, lo=0.0, hi=1.0):
        return jax.random.uniform(self._next(), shape, jnp.bfloat16, lo, hi)
    def permutation(self, n):
        return jax.random.permutation(self._next(), n)


kernel_name = 'recurrent_scan__linear_kernel_hedgehog__dense_activation_relu__prompt'

def _fwd_setup_inputs():
    _rng = _Rng(jax.random.key(int.from_bytes(__import__("os").urandom(4), "little")))
    _w = (lambda a: (lambda t: t.astype(jnp.bfloat16) if jnp.issubdtype(t.dtype, jnp.floating) else t)(jnp.asarray(a)))
    def _A_setup():
        B, S, D, H = 1, 2048, 1024, 32
        Dh = D // H
        return {
            "x": _w((lambda *s: _rng.normal(s) * 0.05)(B, S, D)),
            "wqkv": _w((lambda *s: _rng.normal(s) * 0.05)(D, 3 * D)),
            "w_phi": _w((lambda *s: _rng.normal(s) * 0.05)(H, Dh, Dh) * (Dh ** -0.5)),
            "wo": _w((lambda *s: _rng.normal(s) * 0.05)(D, D)),
        }
    _A_in = _A_setup()

    def _B_setup():
        B, S, D, Dff = 1, 2048, 1024, 3584
        return {
            "x": _w((lambda *s: _rng.normal(s) * 0.05)(B, S, D)),
            "w1": _w((lambda *s: _rng.normal(s) * 0.05)(D, Dff)),
            "w2": _w((lambda *s: _rng.normal(s) * 0.05)(Dff, D)),
        }
    _B_in = _B_setup()

    return {
        "A_x": _A_in["x"],
        "A_wqkv": _A_in["wqkv"],
        "A_w_phi": _A_in["w_phi"],
        "A_wo": _A_in["wo"],
        "B_x": _B_in["x"],
        "B_w1": _B_in["w1"],
        "B_w2": _B_in["w2"],
    }

def _fwd_reference(A_x, A_wqkv, A_w_phi, A_wo, B_x, B_w1, B_w2):
    def _A_ref(x, wqkv, w_phi, wo):
        B, S, D = x.shape
        H = 32; Dh = D // H
        qkv = (lambda x, *d: x.transpose(*d))((x @ wqkv).reshape(B, S, 3, H, Dh), 2, 0, 3, 1, 4)
        q, k, v = qkv[0], qkv[1], qkv[2]
        pq = jnp.einsum("bhsd,hdf->bhsf", q, w_phi)
        pk = jnp.einsum("bhsd,hdf->bhsf", k, w_phi)
        phi_q = jnp.concatenate([_softmax(pq, axis=-1), _softmax(-pq, axis=-1)], axis=-1)
        phi_k = jnp.concatenate([_softmax(pk, axis=-1), _softmax(-pk, axis=-1)], axis=-1)
        kv = jnp.einsum("bhsf,bhsd->bhfd", phi_k, v)
        z  = jnp.einsum("bhsf->bhf", phi_k)
        num = jnp.einsum("bhqf,bhfd->bhqd", phi_q, kv)
        den = jnp.einsum("bhqf,bhf->bhq", phi_q, z)[..., None] + 1e-6
        o = num / den
        return (lambda x, *d: x.transpose(*d))(o, 0, 2, 1, 3).reshape(B, S, D) @ wo

    def _B_ref(x, w1, w2):
        h = jnp.einsum("bsd,df->bsf", x, w1)
        zero = jnp.zeros_like(h)
        h = jnp.maximum(h, zero)
        return jnp.einsum("bsf,fd->bsd", h, w2)

    x = A_x
    xn = _layernorm(x, axis=-1)
    s = _A_ref(xn, A_wqkv, A_w_phi, A_wo)
    g = _silu(_B_ref(xn, B_w1, B_w2))
    return x + s * g


def setup_inputs():
    _inp = _fwd_setup_inputs()
    _gk = jax.random.fold_in(jax.random.key(int.from_bytes(__import__("os").urandom(4), "little")), 2**31 - 1)
    _shapes = [[1, 2048, 1024]]
    _dtypes = ['bfloat16']
    _gks = jax.random.split(_gk, len(_shapes))
    _gs = [jax.random.normal(k, s, dtype=jnp.dtype(d)) * 0.05 for k, s, d in zip(_gks, _shapes, _dtypes)]
    _inp["grad_out"] = _gs[0]
    return _inp

def reference(A_x, A_wqkv, A_w_phi, A_wo, B_w1, B_w2, B_x, grad_out):
    _const = dict(B_x=B_x)
    def _f(*_d):
        return _fwd_reference(**{'A_x': _d[0], 'A_wqkv': _d[1], 'A_w_phi': _d[2], 'A_wo': _d[3], 'B_w1': _d[4], 'B_w2': _d[5], **_const})
    _out, _vjp = jax.vjp(_f, A_x, A_wqkv, A_w_phi, A_wo, B_w1, B_w2)
    _grads = _vjp(grad_out)
    _out0 = jnp.asarray(_out)
    return (_out0, *[jnp.asarray(_g) for _g in _grads])
```

```python
import jax
import jax.numpy as jnp
import jax.experimental.pallas as pl
import jax.experimental.pallas.tpu as pltpu

S = 2048
D = 1024
H = 32
DH = 32
DFF = 3584
NPAIR = H // 2
MR = 80
T = 256
NT = S // T
T2 = 512
NT2 = S // T2
CJ = 256
NJ = DFF // CJ
CG = 256
NG = D // CG
CO = 128
LN_EPS = 1e-5
DEN_EPS = 1e-6

F32 = jnp.float32
BF16 = jnp.bfloat16

_NN = (((1,), (0,)), ((), ()))
_NT = (((1,), (1,)), ((), ()))
_TN = (((0,), (0,)), ((), ()))
_TT = (((0,), (1,)), ((), ()))


def _dot(a, b, dn):
    return jax.lax.dot_general(a, b, dn, preferred_element_type=F32)


def _dual_softmax(p, n):
    nh = p.shape[0] // DH
    p3 = p.reshape(nh, DH, n)
    mx = jnp.max(p3, axis=1, keepdims=True)
    mn = jnp.min(p3, axis=1, keepdims=True)
    e1 = jnp.exp(p3 - mx)
    e2 = jnp.exp(mn - p3)
    r1 = 1.0 / jnp.sum(e1, axis=1, keepdims=True)
    r2 = 1.0 / jnp.sum(e2, axis=1, keepdims=True)
    phi = jnp.concatenate([(e1 * r1).astype(BF16), (e2 * r2).astype(BF16)], axis=1)
    return phi.reshape(nh * 2 * DH, n)


def _dual_softmax_bwd(dphi, phi, n):
    d4 = dphi.reshape(4, DH, n)
    a4 = phi.astype(F32).reshape(4, DH, n)
    t = d4 * a4
    ssum = jnp.sum(t, axis=1, keepdims=True)
    u = t - a4 * ssum
    u = u.reshape(2, 2, DH, n)
    return (u[:, 0] - u[:, 1]).reshape(2 * DH, n)


def _round_bf16(x):
    u = pltpu.bitcast(x, jnp.uint32)
    u = (u + jnp.uint32(0x7FFF) + ((u >> 16) & jnp.uint32(1))) & jnp.uint32(0xFFFF0000)
    return pltpu.bitcast(u, F32)


def _pair_mask():
    r = jax.lax.broadcasted_iota(jnp.int32, (MR, 128), 0)
    c = jax.lax.broadcasted_iota(jnp.int32, (MR, 128), 1)
    rh = jnp.where(r < 64, r // 32, (r - 64) // 8)
    return rh == (c // 64)


def _kernel(x_hbm, wqkv_hbm, wphi_hbm, wo_hbm, w1_hbm, w2_hbm, go_hbm,
            out_hbm, gx_hbm, dwqkv_hbm, dwphi_hbm, dwo_hbm, dw1_hbm, dw2_hbm,
            x_v, go_v, wqkv_v, wphi_v, wo_v, w1_v, w2_v,
            weff_v, wbd_v, xn_v, rstd_v, dlt_v, phik_v, b_v,
            acc_v, l6_v, dd_v,
            h_v, df_v, ds_v, ot_v, dpq_v, dxn_v,
            phiq_v, a_v, rden_v, dhp_v, xsa_v, xsb_v,
            ostage_v, ostage2_v, st1_v, st2_v, stq_v, sto_v, dwphi_v, dwbd_v,
            sem_x, sem_go, sem_w, sem_w1, sem_o, sem_o2, sem_s1, sem_s2, sem_sq, sem_so, sem_p):

    dpk_v = h_v.at[0:D, 0:S]
    dvt_v = h_v.at[D:2 * D, 0:S]

    def x_copy(t):
        return pltpu.make_async_copy(x_hbm.at[pl.ds(t * T, T)], x_v.at[pl.ds(t * T, T)], sem_x.at[t])

    go_copy = pltpu.make_async_copy(go_hbm, go_v, sem_go.at[0])

    HC = D // 2

    def wqkv_copy(i, c):
        return pltpu.make_async_copy(wqkv_hbm.at[:, pl.ds(i * D + c * HC, HC)],
                                     wqkv_v.at[i, :, pl.ds(c * HC, HC)], sem_w.at[i * 2 + c])

    wphi_copy = pltpu.make_async_copy(wphi_hbm, wphi_v, sem_w.at[6])
    wo_copy = pltpu.make_async_copy(wo_hbm, wo_v, sem_w.at[7])
    w2_copy = pltpu.make_async_copy(w2_hbm, w2_v, sem_w.at[8])

    def w1_copy(j):
        return pltpu.make_async_copy(w1_hbm.at[:, pl.ds(j * CJ, CJ)], w1_v.at[j], sem_w1.at[j])

    x_copy(0).start()
    x_copy(1).start()
    wqkv_copy(2, 0).start()

    x_v[S:S + T, :] = jnp.zeros((T, D), BF16)
    acc_v[...] = jnp.zeros_like(acc_v)
    b_v[:, 64:MR, :] = jnp.ones((NPAIR, MR - 64, S), BF16)

    def layernorm(t, stage):
        r0 = t * T if isinstance(t, int) else pl.multiple_of(t * T, T)
        LC = 64
        for c in range(T // LC):
            rows = pl.ds(r0 + c * LC, LC)
            x = x_v[rows, :].astype(F32)
            m = jnp.mean(x, axis=-1, keepdims=True)
            xc = x - m
            var = jnp.mean(xc * xc, axis=-1, keepdims=True)
            mb = _round_bf16(m)
            r = jax.lax.rsqrt(var + LN_EPS)
            dl = (m - mb) * r
            xn = (xc * r + dl).astype(BF16)
            dlt_v[rows, :] = dl
            xn_v[rows, :] = xn
            if stage is not None:
                stage[c * LC:(c + 1) * LC, :] = xn
            rstd_v[rows, :] = r

    def make_weff(i):
        for b in range(8):
            w = _dot(wbd_v[b], wqkv_v[i, :, b * 128:(b + 1) * 128], _TT)
            weff_v[i * D + b * 128:i * D + (b + 1) * 128, :] = w.astype(BF16)

    def key_feats(xn, rows, n):
        pk = _dot(weff_v[D:2 * D, :], xn, _NT)
        phik_v[:, rows] = _dual_softmax(pk, n)

    def kv_sums(rows):
        for p in range(NPAIR):
            acc_v[p] += _dot(b_v[p, :, rows], phik_v[p * 128:(p + 1) * 128, rows], _NT)

    def ln0_body(t, carry):
        x_copy(t).wait()

        @pl.when(t == 0)
        def _():
            wphi_copy.start()
            wqkv_copy(2, 1).start()

        layernorm(t, None)
        return carry

    jax.lax.fori_loop(0, 2, ln0_body, 0)
    PPC = HC // 64

    def vt0_body(c, carry):
        wqkv_copy(2, c).wait()

        @pl.when(c == 0)
        def _():
            wqkv_copy(1, 0).start()
            wqkv_copy(1, 1).start()
            x_copy(2).start()

        cols = pl.ds(pl.multiple_of(c * HC, HC), HC)
        vt = _dot(wqkv_v[2, :, cols], xn_v[0:2 * T, :], _TT).astype(BF16)
        b_v[pl.ds(c * PPC, PPC), 0:64, 0:2 * T] = vt.reshape(PPC, 64, 2 * T)
        return carry

    jax.lax.fori_loop(0, 2, vt0_body, 0)
    wphi_copy.wait()
    wqkv_copy(1, 0).wait()
    wqkv_copy(1, 1).wait()
    x_copy(2).wait()
    for t in range(3, NT):
        x_copy(t).start()
    for j in range(NJ):
        w1_copy(j).start()
    w2_copy.start()
    go_copy.start()
    rr = jax.lax.broadcasted_iota(jnp.int32, (128, 128), 0)
    cc_ = jax.lax.broadcasted_iota(jnp.int32, (128, 128), 1)
    bd_mask = (rr // DH) == (cc_ // DH)
    for b in range(8):
        wc = wphi_v[b * 128:(b + 1) * 128, :].astype(F32)
        wt = jnp.concatenate([wc, wc, wc, wc], axis=1)
        wbd_v[b] = jnp.where(bd_mask, wt, 0.0).astype(BF16)
    make_weff(1)
    layernorm(2, xsa_v)
    key_feats(xn_v[0:2 * T, :], pl.ds(0, 2 * T), 2 * T)
    kv_sums(pl.ds(0, 2 * T))

    def p1_tile(t, cur, nxt):
        r0 = pl.multiple_of(t * T, T)
        rows = pl.ds(r0, T)
        key_feats(cur[...], rows, T)
        vt = _dot(wqkv_v[2], cur[...], _TT).astype(BF16)
        b_v[:, 0:64, rows] = vt.reshape(NPAIR, 64, T)
        kv_sums(rows)
        layernorm(t + 1, nxt)

    def p1_body(k, carry):
        x_copy(2 * k + 1).wait()

        @pl.when(2 * k + 2 < NT)
        def _():
            x_copy(2 * k + 2).wait()

        p1_tile(2 * k, xsa_v, xsb_v)
        p1_tile(2 * k + 1, xsb_v, xsa_v)
        return carry

    jax.lax.fori_loop(1, NT // 2, p1_body, 0)

    pm = _pair_mask()
    for p in range(NPAIR):
        l6_v[p] = jnp.where(pm, acc_v[p], 0.0).astype(BF16)
    acc_v[...] = jnp.zeros_like(acc_v)

    for j in range(NJ):
        w1_copy(j).wait()
    w2_copy.wait()
    go_copy.wait()
    wqkv_copy(0, 0).start()
    wqkv_copy(0, 1).start()
    wo_copy.start()

    def out_copy(t, slot):
        return pltpu.make_async_copy(ostage2_v.at[slot], out_hbm.at[pl.ds(t * T2, T2)], sem_o2.at[slot])

    def gx_copy(t, slot):
        return pltpu.make_async_copy(ostage_v.at[slot], gx_hbm.at[pl.ds(t * T, T)], sem_o.at[slot])

    def p2a_body(t, carry):
        r0 = pl.multiple_of(t * T, T)
        rows = pl.ds(r0, T)
        for j in range(NJ):
            hp = _dot(xn_v[rows, :], w1_v[j], _NN)
            hr = jnp.where(hp < 0.0, -0.0, jnp.abs(hp))
            h_v[rows, j * CJ:(j + 1) * CJ] = hr.astype(BF16)
        f = _dot(h_v[rows, :], w2_v[...], _NN)
        go = go_v[rows, :].astype(F32)
        sig = 0.5 * jnp.tanh(0.5 * f) + 0.5
        g = f * sig
        dxn_v[rows, :] = g
        ds_v[rows, :] = (go * g).astype(BF16)
        df_v[rows, :] = (go * (sig * (1.0 + f * (1.0 - sig)))).astype(BF16)
        return carry

    jax.lax.fori_loop(0, NT, p2a_body, 0)

    wqkv_copy(0, 0).wait()
    wqkv_copy(0, 1).wait()
    wo_copy.wait()
    make_weff(0)

    def p2_body(t, carry):
        r0 = pl.multiple_of(t * T2, T2)
        rows = pl.ds(r0, T2)
        slot = t % 2

        @pl.when(t >= 2)
        def _():
            out_copy(t - 2, slot).wait()

        pq = _dot(weff_v[0:D, :], xn_v[rows, :], _NT)
        phiq_v[...] = _dual_softmax(pq, T2)
        for p in range(NPAIR):
            res = _dot(l6_v[p], phiq_v[p * 128:(p + 1) * 128, :], _NN)
            num = res[0:64].reshape(2, 4, 8, T2)
            rd = 1.0 / (res[64:MR].reshape(2, 1, 8, T2) + DEN_EPS)
            ot_v[p * 64:(p + 1) * 64, rows] = (num * rd).reshape(64, T2).astype(BF16)
            rden_v[p] = rd.reshape(16, T2)
        s = _dot(ot_v[:, rows], wo_v[...], _TN)
        ostage2_v[slot] = (x_v[rows, :].astype(F32) + s * dxn_v[rows, :]).astype(BF16)
        df_v[rows, :] = (df_v[rows, :].astype(F32) * s).astype(BF16)
        dot_ = _dot(wo_v[...], ds_v[rows, :], _NT)
        for p in range(NPAIR):
            do4 = dot_[p * 64:(p + 1) * 64].reshape(2, 4, 8, T2)
            o4 = ot_v[p * 64:(p + 1) * 64, rows].astype(F32).reshape(2, 4, 8, T2)
            rd = rden_v[p].reshape(2, 1, 8, T2)
            dnum = do4 * rd
            c = jnp.sum(dnum * o4, axis=1, keepdims=True)
            c = jnp.sum(c, axis=2, keepdims=True)
            dden = jnp.broadcast_to(c * (-0.125), (2, 1, 8, T2))
            a_v[p, 0:64, :] = dnum.reshape(64, T2).astype(BF16)
            a_v[p, 64:MR, :] = dden.reshape(16, T2).astype(BF16)
        for p in range(NPAIR):
            dphi = _dot(l6_v[p], a_v[p], _TN)
            dpq_v[p * 64:(p + 1) * 64, rows] = _dual_softmax_bwd(
                dphi, phiq_v[p * 128:(p + 1) * 128, :], T2).astype(BF16)
            acc_v[p] += _dot(a_v[p], phiq_v[p * 128:(p + 1) * 128, :], _NT)
        out_copy(t, slot).start()
        return carry

    jax.lax.fori_loop(0, NT2, p2_body, 0)

    for p in range(NPAIR):
        dd_v[p] = jnp.where(pm, acc_v[p], 0.0).astype(BF16)

    def dw1_copy(j, slot):
        return pltpu.make_async_copy(st1_v.at[slot], dw1_hbm.at[:, pl.ds(j * CJ, CJ)], sem_s1.at[slot])

    def dw2_copy(j, slot):
        return pltpu.make_async_copy(st2_v.at[slot], dw2_hbm.at[pl.ds(j * CJ, CJ), :], sem_s2.at[slot])

    def p3_body(j, carry):
        c0 = pl.multiple_of(j * CJ, CJ)
        cols = pl.ds(c0, CJ)
        slot = j % 2

        @pl.when(j >= 2)
        def _():
            dw1_copy(j - 2, slot).wait()
            dw2_copy(j - 2, slot).wait()

        dh = _dot(df_v[...], w2_v[cols, :], _NT)
        hb = pltpu.bitcast(h_v[:, cols].astype(F32), jnp.int32)
        dhp_v[...] = jnp.where(hb > 0, dh, jnp.where(hb == 0, 0.5 * dh, 0.0)).astype(BF16)
        st2_v[slot] = _dot(h_v[:, cols], df_v[...], _TN).astype(BF16)
        dxn_v[...] = jnp.where(j > 0, dxn_v[...], 0.0) + _dot(dhp_v[...], w1_v[j], _NT)
        st1_v[slot] = _dot(xn_v[0:S, :], dhp_v[...], _TN).astype(BF16)
        dw2_copy(j, slot).start()
        dw1_copy(j, slot).start()
        return carry

    jax.lax.fori_loop(0, NJ, p3_body, 0)

    def dwo_copy(i, slot):
        return pltpu.make_async_copy(sto_v.at[slot], dwo_hbm.at[:, pl.ds(i * CO, CO)], sem_so.at[slot])

    def dwqkv_copy(i, slot):
        return pltpu.make_async_copy(stq_v.at[slot], dwqkv_hbm.at[:, pl.ds(i * CG, CG)], sem_sq.at[slot])

    def feat_grads(which, i, dp_ref, slot, first):
        c0 = pl.multiple_of(i * CG, CG)
        g = _dot(xn_v[0:S, :], dp_ref[pl.ds(c0, CG), :], _TT).astype(BF16)
        for bb in range(CG // 128):
            b = i * (CG // 128) + bb
            gb = g[:, bb * 128:(bb + 1) * 128]
            stq_v[slot, :, bb * 128:(bb + 1) * 128] = _dot(gb, wbd_v[b], _NT).astype(BF16)
            wcols = pl.ds(pl.multiple_of(b * 128, 128), 128)
            dw = _dot(wqkv_v[which, :, wcols], gb, _TN)
            if first:
                dwbd_v[b] = dw
            else:
                dwbd_v[b] += dw

    def key_bwd(t):
        r0 = pl.multiple_of(t * T2, T2)
        rows = pl.ds(r0, T2)
        for p in range(NPAIR):
            dvt_v[p * 64:(p + 1) * 64, rows] = _dot(
                dd_v[p, 0:64, :], phik_v[p * 128:(p + 1) * 128, rows], _NN).astype(BF16)
        for p in range(NPAIR):
            dphi = _dot(dd_v[p], b_v[p, :, rows], _TN)
            dpk_v[p * 64:(p + 1) * 64, rows] = _dual_softmax_bwd(
                dphi, phik_v[p * 128:(p + 1) * 128, rows], T2).astype(BF16)

    def pq_body(i, carry):
        key_bwd(2 * i)
        key_bwd(2 * i + 1)
        feat_grads(0, 2 * i, dpq_v, 2 * i, True)
        feat_grads(0, 2 * i + 1, dpq_v, 2 * i + 1, True)
        dwqkv_copy(2 * i, 2 * i).start()
        dwqkv_copy(2 * i + 1, 2 * i + 1).start()
        return carry

    jax.lax.fori_loop(0, NG // 2, pq_body, 0)

    out_copy(NT2 - 2, (NT2 - 2) % 2).wait()
    out_copy(NT2 - 1, (NT2 - 1) % 2).wait()

    def dwo_chunk(i, slot):
        c0 = pl.multiple_of(i * CO, CO)
        sto_v[slot] = _dot(ot_v[...], ds_v[:, pl.ds(c0, CO)], _NN).astype(BF16)

    def gx_tile(t, slot):
        r0 = pl.multiple_of(t * T, T)
        rows = pl.ds(r0, T)
        dxn = (dxn_v[rows, :] + _dot(dpq_v[:, rows], weff_v[0:D, :], _TN)
               + _dot(dpk_v[:, rows], weff_v[D:2 * D, :], _TN)
               + _dot(dvt_v[:, rows], wqkv_v[2], _TT))
        xn = xn_v[rows, :].astype(F32)
        m1 = jnp.mean(dxn, axis=-1, keepdims=True)
        m2 = jnp.mean(dxn * xn, axis=-1, keepdims=True)
        dx = rstd_v[rows, :] * (dxn - (m1 - dlt_v[rows, :] * m2) - xn * m2)
        ostage_v[slot] = (go_v[rows, :].astype(F32) + dx).astype(BF16)

    def p5a_body(i, carry):
        slot = i % 2

        @pl.when(i >= 2)
        def _():
            gx_copy(i - 2, slot).wait()
            dwo_copy(i - 2, slot).wait()

        dwqkv_copy(i, i).wait()
        dwo_chunk(i, slot)
        gx_tile(i, slot)
        feat_grads(1, i, dpk_v, i, False)
        dwo_copy(i, slot).start()
        gx_copy(i, slot).start()
        dwqkv_copy(NG + i, i).start()
        return carry

    jax.lax.fori_loop(0, NG, p5a_body, 0)

    for h in range(H):
        b, hh = h // 4, h % 4
        dwphi_v[h] = dwbd_v[b, hh * DH:(hh + 1) * DH, hh * DH:(hh + 1) * DH].astype(BF16)
    dwphi_copy = pltpu.make_async_copy(dwphi_v, dwphi_hbm, sem_p.at[0])
    dwphi_copy.start()

    def p5b_body(i, carry):
        slot = i % 2
        gx_copy(NG + i - 2, slot).wait()
        dwo_copy(NG + i - 2, slot).wait()
        dwqkv_copy(NG + i, i).wait()
        dwo_chunk(NG + i, slot)
        gx_tile(NG + i, slot)
        c0 = pl.multiple_of(i * CG, CG)
        stq_v[i] = _dot(xn_v[0:S, :], dvt_v[pl.ds(c0, CG), :], _TT).astype(BF16)
        dwo_copy(NG + i, slot).start()
        gx_copy(NG + i, slot).start()
        dwqkv_copy(2 * NG + i, i).start()
        return carry

    jax.lax.fori_loop(0, NG, p5b_body, 0)

    for j in range(NJ - 2, NJ):
        dw1_copy(j, j % 2).wait()
        dw2_copy(j, j % 2).wait()
    dwphi_copy.wait()
    for i in range(NG - 2, NG):
        dwo_copy(NG + i, i % 2).wait()
        gx_copy(NG + i, i % 2).wait()
    for i in range(NG):
        dwqkv_copy(2 * NG + i, i).wait()


@jax.jit
def pallas_recurrent_scan__linear_kernel_hedgehog__dense_activation_relu__prompt_kernel(
    A_x: jax.Array,
    A_wqkv: jax.Array,
    A_w_phi: jax.Array,
    A_wo: jax.Array,
    B_x: jax.Array,
    B_w1: jax.Array,
    B_w2: jax.Array,
    grad_out: jax.Array,
):
    del B_x
    assert NT == 2 * NG
    x2 = A_x.reshape(S, D)
    go2 = grad_out.reshape(S, D)
    wphi2 = A_w_phi.reshape(H * DH, DH)

    any_spec = pl.BlockSpec(memory_space=pl.ANY)
    out_shape = (
        jax.ShapeDtypeStruct((S, D), BF16),
        jax.ShapeDtypeStruct((S, D), BF16),
        jax.ShapeDtypeStruct((D, 3 * D), BF16),
        jax.ShapeDtypeStruct((H, DH, DH), BF16),
        jax.ShapeDtypeStruct((D, D), BF16),
        jax.ShapeDtypeStruct((D, DFF), BF16),
        jax.ShapeDtypeStruct((DFF, D), BF16),
    )
    V = pltpu.VMEM
    scratch = [
        V((S + T, D), BF16),
        V((S, D), BF16),
        V((3, D, D), BF16),
        V((H * DH, DH), BF16),
        V((D, D), BF16),
        V((NJ, D, CJ), BF16),
        V((DFF, D), BF16),
        V((2 * D, D), BF16),
        V((8, 128, 128), BF16),
        V((S + T, D), BF16),
        V((S + T, 1), F32),
        V((S + T, 1), F32),
        V((2 * D, S), BF16),
        V((NPAIR, MR, S), BF16),
        V((NPAIR, MR, 128), F32),
        V((NPAIR, MR, 128), BF16),
        V((NPAIR, MR, 128), BF16),
        V((S, DFF), BF16),
        V((S, D), BF16),
        V((S, D), BF16),
        V((D, S), BF16),
        V((D, S), BF16),
        V((S, D), F32),
        V((2 * D, T2), BF16),
        V((NPAIR, MR, T2), BF16),
        V((NPAIR, 16, T2), F32),
        V((S, CJ), BF16),
        V((T, D), BF16),
        V((T, D), BF16),
        V((2, T, D), BF16),
        V((2, T2, D), BF16),
        V((2, D, CJ), BF16),
        V((2, CJ, D), BF16),
        V((NG, D, CG), BF16),
        V((2, D, CO), BF16),
        V((H, DH, DH), BF16),
        V((8, 128, 128), F32),
        pltpu.SemaphoreType.DMA((NT,)),
        pltpu.SemaphoreType.DMA((1,)),
        pltpu.SemaphoreType.DMA((9,)),
        pltpu.SemaphoreType.DMA((NJ,)),
        pltpu.SemaphoreType.DMA((2,)),
        pltpu.SemaphoreType.DMA((2,)),
        pltpu.SemaphoreType.DMA((2,)),
        pltpu.SemaphoreType.DMA((2,)),
        pltpu.SemaphoreType.DMA((NG,)),
        pltpu.SemaphoreType.DMA((2,)),
        pltpu.SemaphoreType.DMA((1,)),
    ]
    outs = pl.pallas_call(
        _kernel,
        out_shape=out_shape,
        in_specs=[any_spec] * 7,
        out_specs=(any_spec,) * 7,
        scratch_shapes=scratch,
        compiler_params=pltpu.CompilerParams(vmem_limit_bytes=127 * 1024 * 1024),
    )(x2, A_wqkv, wphi2, A_wo, B_w1, B_w2, go2)
    out, gx, dwqkv, dwphi, dwo, dw1, dw2 = outs
    return (out.reshape(1, S, D), gx.reshape(1, S, D), dwqkv, dwphi, dwo, dw1, dw2)
```
